```python
import os as _os
_os.environ.setdefault("JAX_PLATFORMS", "cpu")
import jax
import jax.numpy as jnp

def _softmax(x, axis=-1):
    return jax.nn.softmax(x, axis=axis)
def _gelu(x):
    return jax.nn.gelu(x, approximate=True)
def _silu(x):
    return jax.nn.silu(x)
def _sigmoid(x):
    return jax.nn.sigmoid(x)
def _layernorm(x, axis=-1, eps=1e-5):
    m = jnp.mean(x, axis=axis, keepdims=True)
    v = jnp.var(x, axis=axis, keepdims=True)
    return (x - m) / jnp.sqrt(v + eps)
def _scatter_add(tgt, idx, src, axis=0):
    return tgt.at[idx].add(src)
def _segment_sum(src, seg, n):
    return jax.ops.segment_sum(src, seg, n)
class _Rng:
    def __init__(self, key):
        self._k = key
    def _next(self):
        self._k, sub = jax.random.split(self._k)
        return sub
    def normal(self, shape):
        return jax.random.normal(self._next(), shape, dtype=jnp.bfloat16)
    def randint(self, lo, hi, shape):
        return jax.random.randint(self._next(), shape, lo, hi, dtype=jnp.int32)
    def uniform(self, shape, lo=0.0, hi=1.0):
        return jax.random.uniform(self._next(), shape, jnp.bfloat16, lo, hi)
    def permutation(self, n):
        return jax.random.permutation(self._next(), n)


kernel_name = 'concat_heads__gqa_block_cached__gqa_block_cached__near_ridge'

def setup_inputs():
    _rng = _Rng(jax.random.key(int.from_bytes(__import__("os").urandom(4), "little")))
    _w = (lambda a: (lambda t: t.astype(jnp.bfloat16) if jnp.issubdtype(t.dtype, jnp.floating) else t)(jnp.asarray(a)))
    def _A_setup():
        B, Sq, D = 16, 144, 448
        Hq, Hkv, Sk, Dh = 16, 8, 1024, 256
        assert Hq % Hkv == 0, (Hq, Hkv)
        return {
            "x": _w((lambda *s: _rng.normal(s) * 0.8)(B, Sq, D)),
            "k_cache": _w((lambda *s: _rng.normal(s) * 0.8)(B, Hkv, Sk, Dh)),
            "v_cache": _w((lambda *s: _rng.normal(s) * 0.05)(B, Hkv, Sk, Dh)),
            "wq": _w((lambda *s: _rng.normal(s) * 0.8)(D, Hq * Dh) * (D ** -0.5)),
            "wo": _w((lambda *s: _rng.normal(s) * 0.05)(Hq * Dh, D) * ((Hq * Dh) ** -0.5)),
        }
    _A_in = _A_setup()

    def _B_setup():
        B, Sq, D = 16, 144, 448
        Hq, Hkv, Sk, Dh = 16, 8, 1024, 256
        assert Hq % Hkv == 0, (Hq, Hkv)
        return {
            "x": _w((lambda *s: _rng.normal(s) * 0.8)(B, Sq, D)),
            "k_cache": _w((lambda *s: _rng.normal(s) * 0.8)(B, Hkv, Sk, Dh)),
            "v_cache": _w((lambda *s: _rng.normal(s) * 0.05)(B, Hkv, Sk, Dh)),
            "wq": _w((lambda *s: _rng.normal(s) * 0.8)(D, Hq * Dh) * (D ** -0.5)),
            "wo": _w((lambda *s: _rng.normal(s) * 0.05)(Hq * Dh, D) * ((Hq * Dh) ** -0.5)),
        }
    _B_in = _B_setup()

    return {
        "A_x": _A_in["x"],
        "A_k_cache": _A_in["k_cache"],
        "A_v_cache": _A_in["v_cache"],
        "A_wq": _A_in["wq"],
        "A_wo": _A_in["wo"],
        "B_x": _B_in["x"],
        "B_k_cache": _B_in["k_cache"],
        "B_v_cache": _B_in["v_cache"],
        "B_wq": _B_in["wq"],
        "B_wo": _B_in["wo"],
    }

def reference(A_x, A_k_cache, A_v_cache, A_wq, A_wo, B_x, B_k_cache, B_v_cache, B_wq, B_wo):
    def _A_ref(x, k_cache, v_cache, wq, wo):
        B, Sq, D = x.shape
        Hq, Dh = 16, 256
        Hkv = k_cache.shape[1]
        rep = Hq // Hkv
        q = (lambda x, *d: x.transpose(*d))((x @ wq).reshape(B, Sq, Hq, Dh), 0, 2, 1, 3)
        k = jnp.repeat(k_cache, rep, axis=1)
        v = jnp.repeat(v_cache, rep, axis=1)
        scores = jnp.einsum("bhqd,bhkd->bhqk", q, k) * (Dh ** -0.5)
        p = _softmax(scores, axis=-1)
        o = jnp.einsum("bhqk,bhkd->bhqd", p, v)
        return (lambda x, *d: x.transpose(*d))(o, 0, 2, 1, 3).reshape(B, Sq, Hq * Dh) @ wo

    def _B_ref(x, k_cache, v_cache, wq, wo):
        B, Sq, D = x.shape
        Hq, Dh = 16, 256
        Hkv = k_cache.shape[1]
        rep = Hq // Hkv
        q = (lambda x, *d: x.transpose(*d))((x @ wq).reshape(B, Sq, Hq, Dh), 0, 2, 1, 3)
        k = jnp.repeat(k_cache, rep, axis=1)
        v = jnp.repeat(v_cache, rep, axis=1)
        scores = jnp.einsum("bhqd,bhkd->bhqk", q, k) * (Dh ** -0.5)
        p = _softmax(scores, axis=-1)
        o = jnp.einsum("bhqk,bhkd->bhqd", p, v)
        return (lambda x, *d: x.transpose(*d))(o, 0, 2, 1, 3).reshape(B, Sq, Hq * Dh) @ wo

    a = _A_ref(A_x, A_k_cache, A_v_cache, A_wq, A_wo)
    b = _B_ref(B_x, B_k_cache, B_v_cache, B_wq, B_wo)
    return jnp.concatenate([a, b], axis=-1)
```

```python
import functools
import jax
import jax.numpy as jnp
from jax import lax
import jax.experimental.pallas as pl
import jax.experimental.pallas.tpu as pltpu

LOG2E = 1.4426950408889634
RB = 288
R3 = 256
NT = (((1,), (1,)), ((), ()))
F32 = jnp.float32
BF16 = jnp.bfloat16


def _kernel(xa, ka, va, wqa, woa, xb, kb, vb, wqb, wob, out_hbm,
            kbuf_a, vbuf_a, kbuf_b, vbuf_b, xbuf, wqbuf, wobuf, qo, obuf,
            kvsem, insem, osem,
            *, B, Hkv, Sq, Dh, D, rep):
    W = rep * Dh
    M = B * Sq
    N = Hkv * W
    MH = M // 2
    NQ = N // 4
    scale = (Dh ** -0.5) * LOG2E
    DM = (D // 128) * 128
    DT = D - DM
    kvbufs = ((ka, kbuf_a), (va, vbuf_a), (kb, kbuf_b), (vb, vbuf_b))

    def kv_copy(i, b, slot):
        src, buf = kvbufs[i]
        return pltpu.make_async_copy(src.at[b], buf.at[slot], kvsem.at[i, slot])

    g0 = (pltpu.make_async_copy(xa.at[pl.ds(0, MH)], xbuf.at[0, pl.ds(0, MH)], insem.at[0]),
          pltpu.make_async_copy(wqa.at[:, pl.ds(0, NQ)], wqbuf.at[0, 0], insem.at[0]))
    g1 = (pltpu.make_async_copy(xa.at[pl.ds(MH, MH)], xbuf.at[0, pl.ds(MH, MH)], insem.at[1]),) + tuple(
          pltpu.make_async_copy(wqa.at[:, pl.ds(c * NQ, NQ)], wqbuf.at[0, c], insem.at[1]) for c in range(1, 4))
    g2 = (pltpu.make_async_copy(xb, xbuf.at[1], insem.at[2]),) + tuple(
          pltpu.make_async_copy(wqb.at[:, pl.ds(c * NQ, NQ)], wqbuf.at[1, c], insem.at[2]) for c in range(4))
    g3 = (pltpu.make_async_copy(woa, wobuf.at[0], insem.at[3]),
          pltpu.make_async_copy(wob, wobuf.at[1], insem.at[3]))

    for c in g0:
        c.start()

    def p1_body(i, carry):
        ab = i // 8
        nq = (i % 8) // 2
        mh = i % 2

        @pl.when(i == 0)
        def _():
            for c in g0:
                c.wait()

        @pl.when(i == 1)
        def _():
            for c in g1:
                c.wait()

        @pl.when(i == 8)
        def _():
            for c in g2:
                c.wait()

        @pl.when(i == 0)
        def _():
            for c in g1:
                c.start()

        @pl.when(i == 1)
        def _():
            for c in g2:
                c.start()

        @pl.when(i == 2)
        def _():
            for t in range(4):
                kv_copy(t, 0, 0).start()

        @pl.when(i == 6)
        def _():
            for t in range(4):
                kv_copy(t, 1, 1).start()

        @pl.when(i == 10)
        def _():
            for c in g3:
                c.start()

        row = pl.multiple_of(mh * MH, 16)
        x = xbuf[ab, pl.ds(row, MH), :]
        q = jnp.dot(x, wqbuf[ab, nq], preferred_element_type=F32) * scale
        qo[ab, nq, pl.ds(row, MH), :] = q.astype(BF16)
        return carry

    lax.fori_loop(0, 16, p1_body, 0)

    def p2_body(b, carry):
        slot = b % 2
        for t in range(4):
            kv_copy(t, 0, slot).wait()
        row = pl.multiple_of(b * Sq, 16)
        units = [(ab, h) for ab in range(2) for h in range(Hkv)]

        def qk(ab, h):
            c0 = (h % 2) * W
            q2 = jnp.concatenate(
                [qo[ab, h // 2, pl.ds(row, Sq), c0 + r * Dh:c0 + (r + 1) * Dh] for r in range(rep)], axis=0)
            k = kvbufs[2 * ab][1][slot, h]
            s = lax.dot_general(q2, k, NT, preferred_element_type=F32)
            ps, ls = [], []
            for r0 in range(0, rep * Sq, RB):
                sb = s[r0:r0 + RB]
                m = jnp.max(sb, axis=-1, keepdims=True)
                l = jnp.sum(jnp.exp2(sb - m), axis=-1, keepdims=True)
                ls.append(m + jnp.log2(l))
            m2 = jnp.concatenate(ls, axis=0)
            return jnp.exp2(s - m2).astype(BF16), None

        def pv(ab, h, p, l):
            v = kvbufs[2 * ab + 1][1][slot, h]
            o = jnp.dot(p, v, preferred_element_type=F32)
            o = o.astype(BF16)
            c0 = (h % 2) * W
            for r in range(rep):
                qo[ab, h // 2, pl.ds(row, Sq), c0 + r * Dh:c0 + (r + 1) * Dh] = o[r * Sq:(r + 1) * Sq]

        def refill(ab):
            @pl.when(b + 2 < B)
            def _():
                kv_copy(2 * ab, b + 2, slot).start()
                kv_copy(2 * ab + 1, b + 2, slot).start()

        cur = qk(*units[0])
        for u in range(len(units)):
            nxt = qk(*units[u + 1]) if u + 1 < len(units) else None
            pv(*units[u], *cur)
            cur = nxt
            if units[u][1] == Hkv - 1:
                refill(units[u][0])
        return carry

    lax.fori_loop(0, B, p2_body, 0)

    n3 = M // R3

    def out_copy(i, slot):
        return pltpu.make_async_copy(obuf.at[slot], out_hbm.at[pl.ds(i * R3, R3)], osem.at[slot])

    for c in g3:
        c.wait()

    def p3_body(i, carry):
        slot = i % 2

        @pl.when(i >= 2)
        def _():
            out_copy(0, slot).wait()

        row = pl.multiple_of(i * R3, 128)
        mains, mids = [], []
        for ab in range(2):
            m0 = 0 if ab == 0 else DT
            t0 = DM if ab == 0 else 0
            ym = None
            yt = None
            for c in range(4):
                o = qo[ab, c, pl.ds(row, R3), :]
                a = lax.dot_general(o, wobuf[ab, m0:m0 + DM, c * NQ:(c + 1) * NQ], NT, preferred_element_type=F32)
                t = lax.dot_general(wobuf[ab, t0:t0 + DT, c * NQ:(c + 1) * NQ], o, NT, preferred_element_type=F32)
                ym = a if ym is None else ym + a
                yt = t if yt is None else yt + t
            mains.append(ym)
            mids.append(yt)
        mid = jnp.concatenate(mids, axis=0).T
        obuf[slot, :, 0:DM] = mains[0].astype(BF16)
        obuf[slot, :, DM:DM + 2 * DT] = mid.astype(BF16)
        obuf[slot, :, DM + 2 * DT:] = mains[1].astype(BF16)
        out_copy(i, slot).start()
        return carry

    lax.fori_loop(0, n3, p3_body, 0)
    out_copy(0, (n3 - 2) % 2).wait()
    out_copy(0, (n3 - 1) % 2).wait()


@jax.jit
def pallas_concat_heads__gqa_block_cached__gqa_block_cached__near_ridge_kernel(
    A_x, A_k_cache, A_v_cache, A_wq, A_wo, B_x, B_k_cache, B_v_cache, B_wq, B_wo):
    B, Sq, D = A_x.shape
    _, Hkv, Sk, Dh = A_k_cache.shape
    Hq = A_wq.shape[1] // Dh
    rep = Hq // Hkv
    N = Hq * Dh
    M = B * Sq
    hbm = pl.BlockSpec(memory_space=pl.ANY)
    kv = pltpu.VMEM((2, Hkv, Sk, Dh), BF16)
    out = pl.pallas_call(
        functools.partial(_kernel, B=B, Hkv=Hkv, Sq=Sq, Dh=Dh, D=D, rep=rep),
        in_specs=[hbm] * 10,
        out_specs=hbm,
        out_shape=jax.ShapeDtypeStruct((M, 2 * D), A_x.dtype),
        scratch_shapes=[
            kv, kv, kv, kv,
            pltpu.VMEM((2, M, D), BF16),
            pltpu.VMEM((2, 4, D, N // 4), BF16),
            pltpu.VMEM((2, D, N), BF16),
            pltpu.VMEM((2, 4, M, N // 4), BF16),
            pltpu.VMEM((2, R3, 2 * D), BF16),
            pltpu.SemaphoreType.DMA((4, 2)),
            pltpu.SemaphoreType.DMA((4,)),
            pltpu.SemaphoreType.DMA((2,)),
        ],
        compiler_params=pltpu.CompilerParams(
            vmem_limit_bytes=120 * 1024 * 1024,
            disable_bounds_checks=True),
    )(A_x.reshape(M, D), A_k_cache, A_v_cache, A_wq, A_wo.T,
      B_x.reshape(M, D), B_k_cache, B_v_cache, B_wq, B_wo.T)
    return out.reshape(B, Sq, 2 * D)
```

```python
import functools

import jax
import jax.numpy as jnp
from jax import lax
import jax.experimental.pallas as pl
import jax.experimental.pallas.tpu as pltpu

LOG2E = 1.4426950408889634
NT = (((1,), (1,)), ((), ()))
F32 = jnp.float32
BF16 = jnp.bfloat16
LANES = 128
R3 = 128
U3 = 2
LA = 2


def _kernel(xa, ka, va, wqa, woa, xb, kb, vb, wqb, wob, out_hbm,
            kbuf_a, vbuf_a, kbuf_b, vbuf_b, xbuf, wqbuf, wobuf, qo, obuf,
            kvsem, insem, osem,
            *, B, Hkv, Sq, Dh, D, rep):
    W = rep * Dh
    M = B * Sq
    MH = M // 2
    MQ = M // 4
    scale = (Dh ** -0.5) * LOG2E
    DM = (D // LANES) * LANES
    DT = D - DM
    kvbufs = ((ka, kbuf_a), (va, vbuf_a), (kb, kbuf_b), (vb, vbuf_b))

    def kv_copy(i, b, slot):
        src, buf = kvbufs[i]
        return pltpu.make_async_copy(src.at[b], buf.at[slot], kvsem.at[i, slot])

    def x_copy(src, ab, r0, nr, g):
        return pltpu.make_async_copy(
            src.at[pl.ds(r0, nr)], xbuf.at[pl.ds(ab * M + r0, nr)], insem.at[g])

    def wq_copy(src, ab, h, g):
        return pltpu.make_async_copy(
            src.at[:, pl.ds(h * W, W)], wqbuf.at[ab * Hkv + h], insem.at[g])

    groups = (
        (x_copy(xa, 0, 0, MQ, 0), wq_copy(wqa, 0, 0, 0)),
        (x_copy(xa, 0, MQ, MQ, 1), wq_copy(wqa, 0, 1, 1)),
        (x_copy(xa, 0, MH, MH, 2), wq_copy(wqa, 0, 2, 2), wq_copy(wqa, 0, 3, 2)),
        tuple(wq_copy(wqa, 0, h, 3) for h in range(4, Hkv)) + (x_copy(xb, 1, 0, M, 3),)
        + tuple(wq_copy(wqb, 1, h, 3) for h in range(Hkv)),
        (pltpu.make_async_copy(woa, wobuf.at[0], insem.at[4]),
         pltpu.make_async_copy(wob, wobuf.at[1], insem.at[4])),
    )
    for g in groups[:4]:
        for c in g:
            c.start()

    def wait_group(g):
        for c in groups[g]:
            c.wait()

    def qproj(xr0, r0, nr, hs):
        x = xbuf[pl.ds(xr0, nr), :]
        w = [wqbuf[h] for h in hs]
        w = w[0] if len(w) == 1 else jnp.concatenate(w, axis=1)
        q = (jnp.dot(x, w, preferred_element_type=F32) * scale).astype(BF16)
        for t, h in enumerate(hs):
            qo[h, pl.ds(r0, nr), :] = q[:, t * W:(t + 1) * W]

    wait_group(0)
    qproj(0, 0, MQ, (0,))
    wait_group(1)
    qproj(0, 0, MQ, (1,))
    qproj(MQ, MQ, MQ, (0, 1))

    def p1_body(j, carry):
        @pl.when(j == 1)
        def _():
            wait_group(2)

        @pl.when(j == 4)
        def _():
            wait_group(3)

        @pl.when(j == 4)
        def _():
            for s in range(2):
                for t in range(4):
                    kv_copy(t, s, s).start()
            for c in groups[4]:
                c.start()

        h0 = j & ~1
        r0 = pl.multiple_of((j & 1) * MH, 16)
        xr0 = pl.multiple_of(jnp.where(j >= Hkv, M, 0) + r0, 16)
        qproj(xr0, r0, MH, (h0, h0 + 1))
        return carry

    lax.fori_loop(1, 2 * Hkv, p1_body, 0)

    def p2_body(b, carry):
        slot = b & 1
        for t in range(4):
            kv_copy(t, 0, slot).wait()
        row = pl.multiple_of(b * Sq, 16)

        def qk(ab, h, r):
            q = qo[ab * Hkv + h, pl.ds(row, Sq), r * Dh:(r + 1) * Dh]
            k = kvbufs[2 * ab][1][slot, h]
            s = lax.dot_general(q, k, NT, preferred_element_type=F32)
            m = jnp.max(s, axis=-1, keepdims=True)
            l = jnp.sum(jnp.exp2(s - m), axis=-1, keepdims=True)
            return jnp.exp2(s - (m + jnp.log2(l))).astype(BF16)

        def pv(ab, h, r, p):
            v = kvbufs[2 * ab + 1][1][slot, h]
            o = jnp.dot(p, v, preferred_element_type=F32)
            qo[ab * Hkv + h, pl.ds(row, Sq), r * Dh:(r + 1) * Dh] = o.astype(BF16)

        def refill(ab):
            @pl.when(b + 2 < B)
            def _():
                kv_copy(2 * ab, b + 2, slot).start()
                kv_copy(2 * ab + 1, b + 2, slot).start()

        heads = [(ab, h, r) for ab in range(2) for h in range(Hkv) for r in range(rep)]
        ps = {u: qk(*heads[u]) for u in range(LA)}
        for u, head in enumerate(heads):
            if u + LA < len(heads):
                ps[u + LA] = qk(*heads[u + LA])
            pv(*head, ps.pop(u))
            if head[1:] == (Hkv - 1, rep - 1):
                refill(head[0])
        return carry

    lax.fori_loop(0, B, p2_body, 0)

    wait_group(4)

    def out_copy(row, c0, nc):
        return pltpu.make_async_copy(
            obuf.at[pl.ds(row, R3), pl.ds(c0, nc)],
            out_hbm.at[pl.ds(row, R3), pl.ds(c0, nc)], osem.at[0])

    def p3_body(i, carry):
        for t in range(U3):
            row = pl.multiple_of((i * U3 + t) * R3, LANES)
            o = [[qo[ab * Hkv + h, pl.ds(row, R3), :] for h in range(Hkv)] for ab in range(2)]
            mids = []
            for ab in range(2):
                t0 = DM if ab == 0 else 0
                y = None
                for h in range(Hkv):
                    a = lax.dot_general(wobuf[ab, t0:t0 + DT, h * W:(h + 1) * W], o[ab][h], NT,
                                        preferred_element_type=F32)
                    y = a if y is None else y + a
                mids.append(y)
            mid = jnp.concatenate(mids, axis=0).T
            obuf[pl.ds(row, R3), DM:DM + 2 * DT] = mid.astype(BF16)
            for ab in range(2):
                m0 = 0 if ab == 0 else DT
                c0 = 0 if ab == 0 else DM + 2 * DT
                y = None
                for h in range(Hkv):
                    a = lax.dot_general(o[ab][h], wobuf[ab, m0:m0 + DM, h * W:(h + 1) * W], NT,
                                        preferred_element_type=F32)
                    y = a if y is None else y + a
                obuf[pl.ds(row, R3), c0:c0 + DM] = y.astype(BF16)
                out_copy(row, c0, DM + 2 * DT if ab == 0 else DM).start()
        return carry

    lax.fori_loop(0, M // (R3 * U3), p3_body, 0)
    pltpu.make_async_copy(obuf, out_hbm, osem.at[0]).wait()


@jax.jit
def pallas_concat_heads__gqa_block_cached__gqa_block_cached__near_ridge_kernel(
    A_x: jax.Array,
    A_k_cache: jax.Array,
    A_v_cache: jax.Array,
    A_wq: jax.Array,
    A_wo: jax.Array,
    B_x: jax.Array,
    B_k_cache: jax.Array,
    B_v_cache: jax.Array,
    B_wq: jax.Array,
    B_wo: jax.Array,
):
    B, Sq, D = A_x.shape
    _, Hkv, Sk, Dh = A_k_cache.shape
    N = A_wq.shape[1]
    rep = N // (Hkv * Dh)
    W = rep * Dh
    M = B * Sq
    assert 2 * (D % LANES) == LANES and Hkv >= 4 and Hkv % 2 == 0 and B >= 2
    assert Sq % 16 == 0 and M % 64 == 0 and M % (R3 * U3) == 0

    hbm = pl.BlockSpec(memory_space=pl.ANY)
    kv = pltpu.VMEM((2, Hkv, Sk, Dh), BF16)
    out = pl.pallas_call(
        functools.partial(_kernel, B=B, Hkv=Hkv, Sq=Sq, Dh=Dh, D=D, rep=rep),
        in_specs=[hbm] * 10,
        out_specs=hbm,
        out_shape=jax.ShapeDtypeStruct((M, 2 * D), A_x.dtype),
        scratch_shapes=[
            kv, kv, kv, kv,
            pltpu.VMEM((2 * M, D), BF16),
            pltpu.VMEM((2 * Hkv, D, W), BF16),
            pltpu.VMEM((2, D, N), BF16),
            pltpu.VMEM((2 * Hkv, M, W), BF16),
            pltpu.VMEM((M, 2 * D), BF16),
            pltpu.SemaphoreType.DMA((4, 2)),
            pltpu.SemaphoreType.DMA((5,)),
            pltpu.SemaphoreType.DMA((1,)),
        ],
        compiler_params=pltpu.CompilerParams(
            vmem_limit_bytes=112 * 1024 * 1024,
            disable_bounds_checks=True),
    )(A_x.reshape(M, D), A_k_cache, A_v_cache, A_wq, A_wo.T,
      B_x.reshape(M, D), B_k_cache, B_v_cache, B_wq, B_wo.T)
    return out.reshape(B, Sq, 2 * D)
```

```python
import functools

import jax
import jax.numpy as jnp
from jax import lax
import jax.experimental.pallas as pl
import jax.experimental.pallas.tpu as pltpu

LOG2E = 1.4426950408889634
NT = (((1,), (1,)), ((), ()))
F32 = jnp.float32
BF16 = jnp.bfloat16
LANES = 128
R3 = 128
U3 = 2
LA = 2


def _kernel(xa, ka, va, wqa, woa, xb, kb, vb, wqb, wob, out_hbm,
            kbuf_a, vbuf_a, kbuf_b, vbuf_b, xbuf, wqbuf, wobuf, qo, obuf,
            kvsem, insem, osem,
            *, B, Hkv, Sq, Dh, D, rep):
    W = rep * Dh
    M = B * Sq
    MH = M // 2
    RA = max(16, MH * 3 // 16 // 16 * 16)
    RB = MH * 5 // 8 // 16 * 16
    scale = (Dh ** -0.5) * LOG2E
    DM = (D // LANES) * LANES
    DT = D - DM
    kvbufs = ((ka, kbuf_a), (va, vbuf_a), (kb, kbuf_b), (vb, vbuf_b))

    def kv_copy(i, b, slot):
        src, buf = kvbufs[i]
        return pltpu.make_async_copy(src.at[b], buf.at[slot], kvsem.at[slot])

    def x_copy(src, ab, r0, nr, g):
        return pltpu.make_async_copy(
            src.at[pl.ds(r0, nr)], xbuf.at[pl.ds(ab * M + r0, nr)], insem.at[g])

    def wq_copy(src, ab, h, g):
        return pltpu.make_async_copy(
            src.at[:, pl.ds(h * W, W)], wqbuf.at[ab * Hkv + h], insem.at[g])

    groups = (
        (x_copy(xa, 0, 0, RA, 0), wq_copy(wqa, 0, 0, 0)),
        (x_copy(xa, 0, RA, RB - RA, 1),),
        (x_copy(xa, 0, RB, MH - RB, 2), wq_copy(wqa, 0, 1, 2)),
        (x_copy(xa, 0, MH, MH, 3), wq_copy(wqa, 0, 2, 3), wq_copy(wqa, 0, 3, 3)),
        tuple(wq_copy(wqa, 0, h, 4) for h in range(4, Hkv)) + (x_copy(xb, 1, 0, M, 4),)
        + tuple(wq_copy(wqb, 1, h, 4) for h in range(Hkv)),
        (pltpu.make_async_copy(woa, wobuf.at[0], insem.at[5]),
         pltpu.make_async_copy(wob, wobuf.at[1], insem.at[5])),
    )
    for g in groups[:5]:
        for c in g:
            c.start()

    def wait_group(g):
        for c in groups[g]:
            c.wait()

    def qproj(xr0, r0, nr, hs):
        x = xbuf[pl.ds(xr0, nr), :]
        w = [wqbuf[h] for h in hs]
        w = w[0] if len(w) == 1 else jnp.concatenate(w, axis=1)
        q = (jnp.dot(x, w, preferred_element_type=F32) * scale).astype(BF16)
        for t, h in enumerate(hs):
            qo[h, pl.ds(r0, nr), :] = q[:, t * W:(t + 1) * W]

    wait_group(0)
    qproj(0, 0, RA, (0,))
    wait_group(1)
    qproj(RA, RA, RB - RA, (0,))
    wait_group(2)
    qproj(0, 0, RB, (1,))
    qproj(RB, RB, MH - RB, (0, 1))

    def p1_body(i, carry):
        @pl.when(i == 0)
        def _():
            wait_group(3)

        @pl.when(i == 2)
        def _():
            wait_group(4)

        @pl.when(i == 2)
        def _():
            for s in range(2):
                for t in range(4):
                    kv_copy(t, s, s).start()
            for c in groups[5]:
                c.start()

        qt = i & 3
        js = 1 + 5 * lax.shift_right_logical(i, 2)
        for j, off, nr in ((js + 1 + qt, 0, MH), (js, qt * (MH // 4), MH // 4)):
            h0 = j & ~1
            r0 = pl.multiple_of((j & 1) * MH + off, 16)
            xr0 = pl.multiple_of(jnp.where(j >= Hkv, M, 0) + r0, 16)
            qproj(xr0, r0, nr, (h0, h0 + 1))
        return carry

    lax.fori_loop(0, (2 * Hkv - 1) // 5 * 4, p1_body, 0)

    def p2_body(b, carry):
        slot = b & 1
        for t in range(4):
            kv_copy(t, b, slot).wait()
        row = pl.multiple_of(b * Sq, 16)

        def qk(ab, h, r):
            q = qo[ab * Hkv + h, pl.ds(row, Sq), r * Dh:(r + 1) * Dh]
            k = kvbufs[2 * ab][1][slot, h]
            s = lax.dot_general(q, k, NT, preferred_element_type=F32)
            m = jnp.max(s, axis=-1, keepdims=True)
            l = jnp.sum(jnp.exp2(s - m), axis=-1, keepdims=True)
            return jnp.exp2(s - (m + jnp.log2(l))).astype(BF16)

        def pv(ab, h, r, p):
            v = kvbufs[2 * ab + 1][1][slot, h]
            o = jnp.dot(p, v, preferred_element_type=F32)
            qo[ab * Hkv + h, pl.ds(row, Sq), r * Dh:(r + 1) * Dh] = o.astype(BF16)

        def refill(ab):
            @pl.when(b + 2 < B)
            def _():
                kv_copy(2 * ab, b + 2, slot).start()
                kv_copy(2 * ab + 1, b + 2, slot).start()

        heads = [(ab, h, r) for ab in range(2) for h in range(Hkv) for r in range(rep)]
        ps = {u: qk(*heads[u]) for u in range(LA)}
        for u, head in enumerate(heads):
            if u + LA < len(heads):
                ps[u + LA] = qk(*heads[u + LA])
            pv(*head, ps.pop(u))
            if head[1:] == (Hkv - 1, rep - 1):
                refill(head[0])
        return carry

    lax.fori_loop(0, B, p2_body, 0)

    wait_group(5)

    def out_copy(row, c0, nc):
        return pltpu.make_async_copy(
            obuf.at[pl.ds(row, R3), pl.ds(c0, nc)],
            out_hbm.at[pl.ds(row, R3), pl.ds(c0, nc)], osem.at[0])

    def p3_body(i, carry):
        for t in range(U3):
            row = pl.multiple_of((i * U3 + t) * R3, LANES)
            o = [[jnp.concatenate([qo[ab * Hkv + h + e, pl.ds(row, R3), :] for e in range(2)], axis=1)
                  for h in range(0, Hkv, 2)] for ab in range(2)]
            mids = []
            for ab in range(2):
                t0 = DM if ab == 0 else 0
                y = None
                for c, oc in enumerate(o[ab]):
                    a = lax.dot_general(wobuf[ab, t0:t0 + DT, c * 2 * W:(c + 1) * 2 * W], oc, NT,
                                        preferred_element_type=F32)
                    y = a if y is None else y + a
                mids.append(y)
            mid = jnp.concatenate(mids, axis=0).T
            obuf[pl.ds(row, R3), DM:DM + 2 * DT] = mid.astype(BF16)
            for ab in range(2):
                m0 = 0 if ab == 0 else DT
                c0 = 0 if ab == 0 else DM + 2 * DT
                y = None
                for c, oc in enumerate(o[ab]):
                    a = lax.dot_general(oc, wobuf[ab, m0:m0 + DM, c * 2 * W:(c + 1) * 2 * W], NT,
                                        preferred_element_type=F32)
                    y = a if y is None else y + a
                obuf[pl.ds(row, R3), c0:c0 + DM] = y.astype(BF16)
                out_copy(row, c0, DM + 2 * DT if ab == 0 else DM).start()
        return carry

    lax.fori_loop(0, M // (R3 * U3), p3_body, 0)
    pltpu.make_async_copy(obuf, out_hbm, osem.at[0]).wait()


@jax.jit
def pallas_concat_heads__gqa_block_cached__gqa_block_cached__near_ridge_kernel(
    A_x: jax.Array,
    A_k_cache: jax.Array,
    A_v_cache: jax.Array,
    A_wq: jax.Array,
    A_wo: jax.Array,
    B_x: jax.Array,
    B_k_cache: jax.Array,
    B_v_cache: jax.Array,
    B_wq: jax.Array,
    B_wo: jax.Array,
):
    B, Sq, D = A_x.shape
    _, Hkv, Sk, Dh = A_k_cache.shape
    N = A_wq.shape[1]
    rep = N // (Hkv * Dh)
    W = rep * Dh
    M = B * Sq
    assert 2 * (D % LANES) == LANES and Hkv % 2 == 0 and (2 * Hkv - 1) % 5 == 0 and B >= 2
    assert Sq % 16 == 0 and M % 128 == 0 and M % (R3 * U3) == 0

    hbm = pl.BlockSpec(memory_space=pl.ANY)
    kv = pltpu.VMEM((2, Hkv, Sk, Dh), BF16)
    out = pl.pallas_call(
        functools.partial(_kernel, B=B, Hkv=Hkv, Sq=Sq, Dh=Dh, D=D, rep=rep),
        in_specs=[hbm] * 10,
        out_specs=hbm,
        out_shape=jax.ShapeDtypeStruct((M, 2 * D), A_x.dtype),
        scratch_shapes=[
            kv, kv, kv, kv,
            pltpu.VMEM((2 * M, D), BF16),
            pltpu.VMEM((2 * Hkv, D, W), BF16),
            pltpu.VMEM((2, D, N), BF16),
            pltpu.VMEM((2 * Hkv, M, W), BF16),
            pltpu.VMEM((M, 2 * D), BF16),
            pltpu.SemaphoreType.DMA((2,)),
            pltpu.SemaphoreType.DMA((6,)),
            pltpu.SemaphoreType.DMA((1,)),
        ],
        compiler_params=pltpu.CompilerParams(
            vmem_limit_bytes=112 * 1024 * 1024,
            disable_bounds_checks=True,
            disable_semaphore_checks=True),
    )(A_x.reshape(M, D), A_k_cache, A_v_cache, A_wq, A_wo.T,
      B_x.reshape(M, D), B_k_cache, B_v_cache, B_wq, B_wo.T)
    return out.reshape(B, Sq, 2 * D)
```

```python
import functools

import jax
import jax.numpy as jnp
from jax import lax
import jax.experimental.pallas as pl
import jax.experimental.pallas.tpu as pltpu

LOG2E = 1.4426950408889634
NT = (((1,), (1,)), ((), ()))
F32 = jnp.float32
BF16 = jnp.bfloat16
LANES = 128
LA = 1
OPA = 7


def _kernel(xa, ka, va, wqa, woa, xb, kb, vb, wqb, wob, out_hbm,
            kbuf_a, vbuf_a, kbuf_b, vbuf_b, xbuf, wqbuf, wobuf, qo, obuf,
            kvsem, insem, osem,
            *, B, Hkv, Sq, Dh, D, rep):
    W = rep * Dh
    M = B * Sq
    MH = M // 2
    RA = MH // 9 // 16 * 16
    RB = MH * 3 // 8 // 16 * 16
    scale = (Dh ** -0.5) * LOG2E
    DM = (D // LANES) * LANES
    DT = D - DM
    kvbufs = ((ka, kbuf_a), (va, vbuf_a), (kb, kbuf_b), (vb, vbuf_b))

    def kv_copy(i, b, slot):
        src, buf = kvbufs[i]
        return pltpu.make_async_copy(src.at[b], buf.at[slot], kvsem.at[slot])

    def x_copy(src, ab, r0, nr, g):
        return pltpu.make_async_copy(
            src.at[pl.ds(r0, nr)], xbuf.at[pl.ds(ab * M + r0, nr)], insem.at[g])

    def wq_copy(src, ab, h, g):
        return pltpu.make_async_copy(
            src.at[:, pl.ds(h * W, W)], wqbuf.at[ab * Hkv + h], insem.at[g])

    def out_copy(b, r0, nr, c0, nc):
        return pltpu.make_async_copy(
            obuf.at[b, pl.ds(r0, nr), pl.ds(c0, nc)],
            out_hbm.at[b, pl.ds(r0, nr), pl.ds(c0, nc)], osem.at[0])

    groups = (
        (x_copy(xa, 0, 0, RA, 0), wq_copy(wqa, 0, 0, 0)),
        (x_copy(xa, 0, RA, RB - RA, 1),),
        (x_copy(xa, 0, RB, MH - RB, 2),),
        tuple(wq_copy(wqa, 0, h, 3) for h in range(1, 4)),
        tuple(wq_copy(wqa, 0, h, 4) for h in range(4, Hkv)) + (x_copy(xa, 0, MH, MH, 4),),
        (x_copy(xb, 1, 0, M, 5),) + tuple(wq_copy(wqb, 1, h, 5) for h in range(Hkv))
        + (pltpu.make_async_copy(woa, wobuf.at[0], insem.at[5]),
           pltpu.make_async_copy(wob, wobuf.at[1], insem.at[5])),
    )
    for g in groups:
        for c in g:
            c.start()

    def wait_group(g):
        for c in groups[g]:
            c.wait()

    def qproj(xr0, r0, nr, hs):
        x = xbuf[pl.ds(xr0, nr), :]
        w = [wqbuf[h] for h in hs]
        w = w[0] if len(w) == 1 else jnp.concatenate(w, axis=1)
        q = (jnp.dot(x, w, preferred_element_type=F32) * scale).astype(BF16)
        for t, h in enumerate(hs):
            qo[h, pl.ds(r0, nr), :] = q[:, t * W:(t + 1) * W]

    def oproj_t(ab, o):
        t0 = DM if ab == 0 else 0
        return lax.dot_general(wobuf[ab, t0:t0 + DT, :], o, NT, preferred_element_type=F32)

    wait_group(0)
    qproj(0, 0, RA, (0,))
    wait_group(1)
    qproj(RA, RA, RB - RA, (0,))
    wait_group(2)
    qproj(RB, RB, MH - RB, (0,))

    def p1_body(i, carry):
        @pl.when(i == 0)
        def _():
            wait_group(3)

        @pl.when(i == 1)
        def _():
            wait_group(4)

        @pl.when(i == 1)
        def _():
            for t in range(4):
                kv_copy(t, 0, 0).start()

        h0 = jnp.where(i >= 3, 2 * i - 2, 2 * i + 2)
        r0 = pl.multiple_of(jnp.where(i >= 3, MH, 0), 16)
        qproj(r0, r0, MH, (h0, h0 + 1))
        hs = jnp.where(i == 0, 1, i - 1)
        rs = pl.multiple_of(jnp.where(i == 0, 0, MH), 16)
        qproj(rs, rs, MH, (hs,))
        return carry

    lax.fori_loop(0, 5, p1_body, 0)
    wait_group(5)
    for t in range(4):
        kv_copy(t, 1, 1).start()

    def p2_body(b, carry):
        slot = b & 1
        for t in range(4):
            kv_copy(t, b, slot).wait()
        row = pl.multiple_of(b * Sq, 16)

        def qk(ab, h, r):
            q = qo[ab * Hkv + h, pl.ds(row, Sq), r * Dh:(r + 1) * Dh]
            k = kvbufs[2 * ab][1][slot, h]
            s = lax.dot_general(q, k, NT, preferred_element_type=F32)
            m = jnp.max(s, axis=-1, keepdims=True)
            l = jnp.sum(jnp.exp2(s - m), axis=-1, keepdims=True)
            return jnp.exp2(s - (m + jnp.log2(l))).astype(BF16)

        def pv(ab, h, r, p):
            v = kvbufs[2 * ab + 1][1][slot, h]
            o = jnp.dot(p, v, preferred_element_type=F32)
            qo[ab * Hkv + h, pl.ds(row, Sq), r * Dh:(r + 1) * Dh] = o.astype(BF16)

        def refill(ab):
            @pl.when(b + 2 < B)
            def _():
                kv_copy(2 * ab, b + 2, slot).start()
                kv_copy(2 * ab + 1, b + 2, slot).start()

        def load_o(ab):
            return jnp.concatenate(
                [qo[ab * Hkv + h, pl.ds(row, Sq), :] for h in range(Hkv)], axis=1)

        def oproj(ab, o):
            m0 = 0 if ab == 0 else DT
            c0 = 0 if ab == 0 else DM + 2 * DT
            y = lax.dot_general(o, wobuf[ab, m0:m0 + DM, :], NT, preferred_element_type=F32)
            obuf[b, :, c0:c0 + DM] = y.astype(BF16)
            out_copy(b, 0, Sq, c0, DM).start()

        qproj(pl.multiple_of(M + row, 16), row, Sq, tuple(range(Hkv, 2 * Hkv)))

        heads = [(ab, h, r) for ab in range(2) for h in range(Hkv) for r in range(rep)]
        ps = {u: qk(*heads[u]) for u in range(LA)}
        mid_a = None
        for u, head in enumerate(heads):
            if u + LA < len(heads):
                ps[u + LA] = qk(*heads[u + LA])
            pv(*head, ps.pop(u))
            if head[1:] == (Hkv - 1, rep - 1):
                refill(head[0])
            if u == Hkv * rep - 1 + OPA:
                o = load_o(0)
                oproj(0, o)
                mid_a = oproj_t(0, o[:LANES])
        o = load_o(1)
        mid = jnp.concatenate([mid_a, oproj_t(1, o[:LANES])], axis=0).T
        obuf[b, 0:LANES, DM:DM + 2 * DT] = mid.astype(BF16)
        out_copy(b, 0, LANES, DM, 2 * DT).start()
        oproj(1, o)
        return carry

    lax.fori_loop(0, B, p2_body, 0)

    SL = Sq - LANES
    mids = []
    for ab in range(2):
        o = jnp.concatenate(
            [jnp.concatenate([qo[ab * Hkv + h, bb * Sq + LANES:(bb + 1) * Sq, :]
                              for h in range(Hkv)], axis=1)
             for bb in range(B)], axis=0)
        mids.append(oproj_t(ab, o))
    mid = jnp.concatenate(mids, axis=0).T.astype(BF16)
    for bb in range(B):
        obuf[bb, LANES:Sq, DM:DM + 2 * DT] = mid[bb * SL:(bb + 1) * SL]
    pltpu.make_async_copy(obuf.at[:, pl.ds(LANES, SL), pl.ds(DM, 2 * DT)],
                          out_hbm.at[:, pl.ds(LANES, SL), pl.ds(DM, 2 * DT)],
                          osem.at[0]).start()
    pltpu.make_async_copy(obuf, out_hbm, osem.at[0]).wait()


@jax.jit
def pallas_concat_heads__gqa_block_cached__gqa_block_cached__near_ridge_kernel(
    A_x: jax.Array,
    A_k_cache: jax.Array,
    A_v_cache: jax.Array,
    A_wq: jax.Array,
    A_wo: jax.Array,
    B_x: jax.Array,
    B_k_cache: jax.Array,
    B_v_cache: jax.Array,
    B_wq: jax.Array,
    B_wo: jax.Array,
):
    B, Sq, D = A_x.shape
    _, Hkv, Sk, Dh = A_k_cache.shape
    N = A_wq.shape[1]
    rep = N // (Hkv * Dh)
    W = rep * Dh
    M = B * Sq
    assert Hkv == 8 and 2 * (D % LANES) == LANES and B % 2 == 0
    assert Sq % 16 == 0 and Sq > LANES and (B * (Sq - LANES)) % LANES == 0

    hbm = pl.BlockSpec(memory_space=pl.ANY)
    kv = pltpu.VMEM((2, Hkv, Sk, Dh), BF16)
    return pl.pallas_call(
        functools.partial(_kernel, B=B, Hkv=Hkv, Sq=Sq, Dh=Dh, D=D, rep=rep),
        in_specs=[hbm] * 10,
        out_specs=hbm,
        out_shape=jax.ShapeDtypeStruct((B, Sq, 2 * D), A_x.dtype),
        scratch_shapes=[
            kv, kv, kv, kv,
            pltpu.VMEM((2 * M, D), BF16),
            pltpu.VMEM((2 * Hkv, D, W), BF16),
            pltpu.VMEM((2, D, N), BF16),
            pltpu.VMEM((2 * Hkv, M, W), BF16),
            pltpu.VMEM((B, Sq, 2 * D), BF16),
            pltpu.SemaphoreType.DMA((2,)),
            pltpu.SemaphoreType.DMA((6,)),
            pltpu.SemaphoreType.DMA((1,)),
        ],
        compiler_params=pltpu.CompilerParams(
            vmem_limit_bytes=112 * 1024 * 1024,
            disable_bounds_checks=True,
            disable_semaphore_checks=True),
    )(A_x.reshape(M, D), A_k_cache, A_v_cache, A_wq, A_wo.T,
      B_x.reshape(M, D), B_k_cache, B_v_cache, B_wq, B_wo.T)
```

```python
import functools

import jax
import jax.numpy as jnp
from jax import lax
import jax.experimental.pallas as pl
import jax.experimental.pallas.tpu as pltpu

LOG2E = 1.4426950408889634
NT = (((1,), (1,)), ((), ()))
F32 = jnp.float32
BF16 = jnp.bfloat16
LANES = 128
LA = 1
OPA = 7


def _kernel(xa, ka, va, wqa, woa, xb, kb, vb, wqb, wob, out_hbm,
            kbuf_a, vbuf_a, kbuf_b, vbuf_b, xbuf, wqbuf, wobuf, qo, obuf,
            kvsem, insem, osem,
            *, B, Hkv, Sq, Dh, D, rep):
    W = rep * Dh
    M = B * Sq
    MH = M // 2
    RA = MH // 9 // 16 * 16
    RB = MH * 3 // 8 // 16 * 16
    scale = (Dh ** -0.5) * LOG2E
    DM = (D // LANES) * LANES
    DT = D - DM
    kvbufs = ((ka, kbuf_a), (va, vbuf_a), (kb, kbuf_b), (vb, vbuf_b))

    def kv_copy(i, b, slot):
        src, buf = kvbufs[i]
        return pltpu.make_async_copy(src.at[b], buf.at[slot], kvsem.at[slot])

    def x_copy(src, ab, r0, nr, g):
        return pltpu.make_async_copy(
            src.at[pl.ds(r0, nr)], xbuf.at[pl.ds(ab * M + r0, nr)], insem.at[g])

    def wq_copy(src, ab, h, g):
        return pltpu.make_async_copy(
            src.at[:, pl.ds(h * W, W)], wqbuf.at[ab * Hkv + h], insem.at[g])

    def out_copy(b, r0, nr, c0, nc):
        return pltpu.make_async_copy(
            obuf.at[b, pl.ds(r0, nr), pl.ds(c0, nc)],
            out_hbm.at[b, pl.ds(r0, nr), pl.ds(c0, nc)], osem.at[0])

    groups = (
        (x_copy(xa, 0, 0, RA, 0), wq_copy(wqa, 0, 0, 0)),
        (x_copy(xa, 0, RA, RB - RA, 1),),
        (x_copy(xa, 0, RB, MH - RB, 2),),
        tuple(wq_copy(wqa, 0, h, 3) for h in range(1, 4)),
        tuple(wq_copy(wqa, 0, h, 4) for h in range(4, Hkv)) + (x_copy(xa, 0, MH, MH, 4),),
        (x_copy(xb, 1, 0, M, 5),) + tuple(wq_copy(wqb, 1, h, 5) for h in range(Hkv))
        + (pltpu.make_async_copy(woa, wobuf.at[0], insem.at[5]),
           pltpu.make_async_copy(wob, wobuf.at[1], insem.at[5])),
    )
    for g in groups:
        for c in g:
            c.start()

    def wait_group(g):
        for c in groups[g]:
            c.wait()

    def qproj(xr0, r0, nr, hs):
        x = xbuf[pl.ds(xr0, nr), :]
        w = [wqbuf[h] for h in hs]
        w = w[0] if len(w) == 1 else jnp.concatenate(w, axis=1)
        q = (jnp.dot(x, w, preferred_element_type=F32) * scale).astype(BF16)
        for t, h in enumerate(hs):
            qo[h, pl.ds(r0, nr), :] = q[:, t * W:(t + 1) * W]

    def oproj_t(ab, o):
        t0 = DM if ab == 0 else 0
        return lax.dot_general(wobuf[ab, t0:t0 + DT, :], o, NT, preferred_element_type=F32)

    wait_group(0)
    qproj(0, 0, RA, (0,))
    wait_group(1)
    qproj(RA, RA, RB - RA, (0,))
    wait_group(2)
    qproj(RB, RB, MH - RB, (0,))

    def p1_body(i, carry):
        @pl.when(i == 0)
        def _():
            wait_group(3)

        @pl.when(i == 1)
        def _():
            wait_group(4)

        @pl.when(i == 1)
        def _():
            for t in range(4):
                kv_copy(t, 0, 0).start()

        h0 = jnp.where(i >= 3, 2 * i - 2, 2 * i + 2)
        r0 = pl.multiple_of(jnp.where(i >= 3, MH, 0), 16)
        qproj(r0, r0, MH, (h0, h0 + 1))
        hs = jnp.where(i == 0, 1, i - 1)
        rs = pl.multiple_of(jnp.where(i == 0, 0, MH), 16)
        qproj(rs, rs, MH, (hs,))
        return carry

    lax.fori_loop(0, 5, p1_body, 0)
    wait_group(5)
    for t in range(4):
        kv_copy(t, 1, 1).start()

    def p2_body(b, carry):
        slot = b & 1
        for t in range(4):
            kv_copy(t, b, slot).wait()
        row = pl.multiple_of(b * Sq, 16)

        def qk(ab, h, r):
            q = qo[ab * Hkv + h, pl.ds(row, Sq), r * Dh:(r + 1) * Dh]
            k = kvbufs[2 * ab][1][slot, h]
            s = lax.dot_general(q, k, NT, preferred_element_type=F32)
            m = jnp.max(s, axis=-1, keepdims=True)
            l = jnp.sum(jnp.exp2(s - m), axis=-1, keepdims=True)
            return jnp.exp2(s - (m + jnp.log2(l))).astype(BF16)

        def pv(ab, h, r, p):
            v = kvbufs[2 * ab + 1][1][slot, h]
            o = jnp.dot(p, v, preferred_element_type=F32)
            qo[ab * Hkv + h, pl.ds(row, Sq), r * Dh:(r + 1) * Dh] = o.astype(BF16)

        def refill(ab):
            @pl.when(b + 2 < B)
            def _():
                kv_copy(2 * ab, b + 2, slot).start()
                kv_copy(2 * ab + 1, b + 2, slot).start()

        def load_o(ab):
            return jnp.concatenate(
                [qo[ab * Hkv + h, pl.ds(row, Sq), :] for h in range(Hkv)], axis=1)

        def oproj(ab, o):
            m0 = 0 if ab == 0 else DT
            c0 = 0 if ab == 0 else DM + 2 * DT
            y = lax.dot_general(o, wobuf[ab, m0:m0 + DM, :], NT, preferred_element_type=F32)
            obuf[b, :, c0:c0 + DM] = y.astype(BF16)
            out_copy(b, 0, Sq, c0, DM).start()

        qproj(pl.multiple_of(M + row, 16), row, Sq, tuple(range(Hkv, 2 * Hkv)))

        heads = [(ab, h, r) for ab in range(2) for h in range(Hkv) for r in range(rep)]
        ps = {u: qk(*heads[u]) for u in range(LA)}
        mid_a = None
        for u, head in enumerate(heads):
            if u + LA < len(heads):
                ps[u + LA] = qk(*heads[u + LA])
            pv(*head, ps.pop(u))
            if head[1:] == (Hkv - 1, rep - 1):
                refill(head[0])
            if u == Hkv * rep - 1 + OPA:
                o = load_o(0)
                oproj(0, o)
                mid_a = oproj_t(0, o[:LANES])
        o = load_o(1)
        mid = jnp.concatenate([mid_a, oproj_t(1, o[:LANES])], axis=0).T
        obuf[b, 0:LANES, DM:DM + 2 * DT] = mid.astype(BF16)
        out_copy(b, 0, LANES, DM, 2 * DT).start()
        oproj(1, o)
        return carry

    lax.fori_loop(0, B, p2_body, 0)

    SL = Sq - LANES
    GB = LANES // SL
    for b0 in range(0, B, GB):
        mids = []
        for ab in range(2):
            o = jnp.concatenate(
                [jnp.concatenate([qo[ab * Hkv + h, bb * Sq + LANES:(bb + 1) * Sq, :]
                                  for h in range(Hkv)], axis=1)
                 for bb in range(b0, b0 + GB)], axis=0)
            mids.append(oproj_t(ab, o))
        mid = jnp.concatenate(mids, axis=0).T.astype(BF16)
        for t in range(GB):
            obuf[b0 + t, LANES:Sq, DM:DM + 2 * DT] = mid[t * SL:(t + 1) * SL]
            out_copy(b0 + t, LANES, SL, DM, 2 * DT).start()
    pltpu.make_async_copy(obuf, out_hbm, osem.at[0]).wait()


@jax.jit
def pallas_concat_heads__gqa_block_cached__gqa_block_cached__near_ridge_kernel(
    A_x: jax.Array,
    A_k_cache: jax.Array,
    A_v_cache: jax.Array,
    A_wq: jax.Array,
    A_wo: jax.Array,
    B_x: jax.Array,
    B_k_cache: jax.Array,
    B_v_cache: jax.Array,
    B_wq: jax.Array,
    B_wo: jax.Array,
):
    B, Sq, D = A_x.shape
    _, Hkv, Sk, Dh = A_k_cache.shape
    N = A_wq.shape[1]
    rep = N // (Hkv * Dh)
    W = rep * Dh
    M = B * Sq
    assert Hkv == 8 and 2 * (D % LANES) == LANES and B % 2 == 0
    assert Sq % 16 == 0 and Sq > LANES and LANES % (Sq - LANES) == 0
    assert (B * (Sq - LANES)) % LANES == 0

    hbm = pl.BlockSpec(memory_space=pl.ANY)
    kv = pltpu.VMEM((2, Hkv, Sk, Dh), BF16)
    return pl.pallas_call(
        functools.partial(_kernel, B=B, Hkv=Hkv, Sq=Sq, Dh=Dh, D=D, rep=rep),
        in_specs=[hbm] * 10,
        out_specs=hbm,
        out_shape=jax.ShapeDtypeStruct((B, Sq, 2 * D), A_x.dtype),
        scratch_shapes=[
            kv, kv, kv, kv,
            pltpu.VMEM((2 * M, D), BF16),
            pltpu.VMEM((2 * Hkv, D, W), BF16),
            pltpu.VMEM((2, D, N), BF16),
            pltpu.VMEM((2 * Hkv, M, W), BF16),
            pltpu.VMEM((B, Sq, 2 * D), BF16),
            pltpu.SemaphoreType.DMA((2,)),
            pltpu.SemaphoreType.DMA((6,)),
            pltpu.SemaphoreType.DMA((1,)),
        ],
        compiler_params=pltpu.CompilerParams(
            vmem_limit_bytes=112 * 1024 * 1024,
            disable_bounds_checks=True,
            disable_semaphore_checks=True),
    )(A_x.reshape(M, D), A_k_cache, A_v_cache, A_wq, A_wo.T,
      B_x.reshape(M, D), B_k_cache, B_v_cache, B_wq, B_wo.T)
```
